```python
import os as _os
_os.environ.setdefault("JAX_PLATFORMS", "cpu")
import jax
import jax.numpy as jnp

def _softmax(x, axis=-1):
    return jax.nn.softmax(x, axis=axis)
def _gelu(x):
    return jax.nn.gelu(x, approximate=True)
def _silu(x):
    return jax.nn.silu(x)
def _sigmoid(x):
    return jax.nn.sigmoid(x)
def _layernorm(x, axis=-1, eps=1e-5):
    m = jnp.mean(x, axis=axis, keepdims=True)
    v = jnp.var(x, axis=axis, keepdims=True)
    return (x - m) / jnp.sqrt(v + eps)
def _scatter_add(tgt, idx, src, axis=0):
    return tgt.at[idx].add(src)
def _segment_sum(src, seg, n):
    return jax.ops.segment_sum(src, seg, n)
class _Rng:
    def __init__(self, key):
        self._k = key
    def _next(self):
        self._k, sub = jax.random.split(self._k)
        return sub
    def normal(self, shape):
        return jax.random.normal(self._next(), shape, dtype=jnp.bfloat16)
    def randint(self, lo, hi, shape):
        return jax.random.randint(self._next(), shape, lo, hi, dtype=jnp.int32)
    def uniform(self, shape, lo=0.0, hi=1.0):
        return jax.random.uniform(self._next(), shape, jnp.bfloat16, lo, hi)
    def permutation(self, n):
        return jax.random.permutation(self._next(), n)


kernel_name = 'standalone__mha_softmax__near_ridge'

def setup_inputs():
    _rng = _Rng(jax.random.key(int.from_bytes(__import__("os").urandom(4), "little")))
    _w = (lambda a: (lambda t: t.astype(jnp.bfloat16) if jnp.issubdtype(t.dtype, jnp.floating) else t)(jnp.asarray(a)))
    B, H, Sq, Sk, D = 8, 32, 304, 2048, 128
    return {
        "q": _w((lambda *s: _rng.normal(s) * 0.4)(B, H, Sq, D)),
        "k": _w((lambda *s: _rng.normal(s) * 0.4)(B, H, Sk, D)),
        "v": _w((lambda *s: _rng.normal(s) * 0.05)(B, H, Sk, D)),
    }

def reference(q, k, v):
    scale = q.shape[-1] ** -0.5
    scores = jnp.einsum("bhqd,bhkd->bhqk", q, k) * scale
    p = _softmax(scores, axis=-1)
    return jnp.einsum("bhqk,bhkd->bhqd", p, v)
```

```python
import numpy as np
import jax
import jax.numpy as jnp
import jax.experimental.pallas as pl
import jax.experimental.pallas.tpu as pltpu

_reciprocal = pltpu.reciprocal if hasattr(pltpu, "reciprocal") else pl.reciprocal

_STAGES = ((1, 6), (2, 7), (4, 9), (8, 24), (4, 1), (2, 1), (2, 1))
_RING = 64
_FIRST_WRITE = 16
_GATE_TILE = 12


def _or_fold(x):
    parts = [x[8 * i:8 * i + 8] for i in range(x.shape[0] // 8)]
    while len(parts) > 1:
        nxt = [parts[i] | parts[i + 1] for i in range(0, len(parts) - 1, 2)]
        if len(parts) % 2:
            nxt.append(parts[-1])
        parts = nxt
    return parts[0]


def _stage_table(stages, n_heads):
    assert sum(u * n for u, n in stages) == n_heads
    u_max = max(u for u, _ in stages)
    main = min(i for i, (u, _) in enumerate(stages) if u == u_max)
    last_main = max(i for i, (u, _) in enumerate(stages) if u == u_max)
    tab, a, prev = [], 0, 0
    for i, (u, n) in enumerate(stages):
        if prev > u:
            assert n == 1
        if i > last_main:
            assert n == 1
        tab.append(dict(U=u, n=n, a0=a, prev=prev, n_norm=max(u, prev)))
        a += u * n
        prev = u
    return tab, u_max, main, last_main


@jax.jit
def pallas_standalone__mha_softmax__near_ridge_kernel(
    q: jax.Array,
    k: jax.Array,
    v: jax.Array,
):
    B, H, Sq, D = q.shape
    Sk = k.shape[2]
    NH = B * H
    NT = Sk // D
    assert D == 128 and Sk % D == 0 and Sq % 16 == 0
    c = float(D ** -0.5 * np.log2(np.e))
    tab, UM, main, last_main = _stage_table(_STAGES, NH)
    NB = _RING
    NS = NB // UM
    a_main = tab[main]["a0"]
    a_tail = tab[last_main]["a0"] + UM * tab[last_main]["n"]
    n_pro = sum(s["n"] for s in tab[:main])
    tail = tab[last_main + 1:]
    assert a_main <= NB <= a_tail and a_main % UM == 0 and NB % UM == 0
    assert (a_tail - a_main) % UM == 0 and NH - a_tail <= UM
    bf = q.dtype

    def kernel(q_hbm, k_hbm, v_hbm, o_hbm, qb, kb, vb, ob, o_c, l_c, z_ref,
               psem, rsem, tsem, osem):
        q32 = qb.bitcast(jnp.uint32)
        k32 = kb.bitcast(jnp.uint32)
        v32 = vb.bitcast(jnp.uint32)
        o32 = ob.bitcast(jnp.uint32)

        def read_heads(h, slot, n, sem):
            pltpu.make_async_copy(q_hbm.at[pl.ds(h, n)], qb.at[pl.ds(slot, n)], sem).start()
            pltpu.make_async_copy(k_hbm.at[pl.ds(h, n)], kb.at[pl.ds(slot, n)], sem).start()
            pltpu.make_async_copy(v_hbm.at[pl.ds(h, n)], vb.at[pl.ds(slot, n)], sem).start()

        def wait_heads(slot, n, sem):
            pltpu.make_async_copy(qb.at[pl.ds(slot, n)], qb.at[pl.ds(slot, n)], sem).wait()
            pltpu.make_async_copy(kb.at[pl.ds(slot, n)], kb.at[pl.ds(slot, n)], sem).wait()
            pltpu.make_async_copy(vb.at[pl.ds(slot, n)], vb.at[pl.ds(slot, n)], sem).wait()

        def write_heads(h, n):
            pltpu.make_async_copy(ob.at[pl.ds(h + UM, n)], o_hbm.at[pl.ds(h, n)], osem.at[0]).start()

        def read_tail():
            for ti, t in enumerate(tail):
                read_heads(t["a0"], t["a0"] % NB, t["U"], tsem.at[ti])

        pb = 0
        for s in tab[:main]:
            for i in range(s["n"]):
                h0 = s["a0"] + i * s["U"]
                read_heads(h0, h0, s["U"], psem.at[pb])
                pb += 1
        for h0 in range(a_main, min(NB, a_tail), UM):
            read_heads(h0, h0 % NB, UM, rsem.at[(h0 // UM) % NS])

        def scores(q_bits, k_bits):
            qh = pltpu.bitcast(q_bits, bf)
            kh = pltpu.bitcast(k_bits, bf)
            s = jax.lax.dot_general(qh, kh, (((1,), (1,)), ((), ())),
                                    preferred_element_type=jnp.float32)
            return s, jnp.max(s, axis=1, keepdims=True)

        def weighted_values(s, m, v_bits):
            vh = pltpu.bitcast(v_bits, bf)
            p = jnp.exp2((s - m) * c)
            lp = p[:, 0:D]
            for j in range(1, NT):
                lp = lp + p[:, D * j:D * j + D]
            o = jnp.dot(p.astype(bf), vh, preferred_element_type=jnp.float32)
            return o, lp

        def normalise(o, lp):
            l = jnp.sum(lp, axis=1, keepdims=True)
            r = _reciprocal(l, approx=True)
            r = r * (2.0 - l * r)
            return (o * r).astype(bf)

        o_c[...] = jnp.zeros_like(o_c)
        l_c[...] = jnp.ones_like(l_c)
        z_ref[...] = jnp.zeros_like(z_ref)

        def block(si, i, pro_idx):
            st = tab[si]
            U, n_norm, prev = st["U"], st["n_norm"], st["prev"]
            a = st["a0"] + i * U
            static = isinstance(a, int)
            slot = a % NB
            if si < main:
                wait_heads(slot, U, psem.at[pro_idx])
            elif si > last_main:
                wait_heads(slot, U, tsem.at[si - last_main - 1])
            else:
                wait_heads(slot, U, rsem.at[(a // UM) % NS])

            if static:
                n_prev = prev if i == 0 else U
                idx = [(a - n_prev + j + UM) if j < n_prev else j for j in range(n_norm)]
            else:
                base_a = jnp.where(i == 0, st["a0"] - prev + UM, a - U + UM)
                base_b = jnp.where(i == 0, 0, a - U + UM)
                idx = [(base_a + j) if j < prev else (base_b + j) for j in range(n_norm)]
            z = z_ref[...]
            gates = {}
            for j in range(n_norm):
                ob[idx[j]] = normalise(o_c[j], l_c[j])
                g = _or_fold(o32[idx[j]]) & z
                tgt = min(j, U - 1)
                gates[tgt] = g if tgt not in gates else (gates[tgt] | g)

            t0 = (D // 2) * _GATE_TILE
            for h in range(U):
                kk = k32[slot + h]
                if h in gates:
                    kk = jnp.concatenate([kk[:t0], kk[t0:t0 + 8] | gates[h], kk[t0 + 8:]], axis=0)
                s, m = scores(q32[slot + h], kk)
                o, lp = weighted_values(s, m, v32[slot + h])
                o_c[h] = o
                l_c[h] = lp

            def refill():
                read_heads(a + NB, slot, U, rsem.at[((a + NB) // UM) % NS])

            if static:
                if a + NB < a_tail:
                    refill()
                elif a + NB == a_tail and tail:
                    read_tail()
            else:
                last_a = st["a0"] + (st["n"] - 1) * U
                if last_a + NB < a_tail:
                    refill()
                else:
                    if st["a0"] + NB < a_tail:
                        pl.when(a + NB < a_tail)(refill)
                    if tail and st["a0"] + NB <= a_tail <= last_a + NB:
                        pl.when(a + NB == a_tail)(read_tail)

            if si == main:
                iw = min(_FIRST_WRITE, st["n"] - 1)
                aw = st["a0"] + iw * U
                if static:
                    if i == iw and aw > 0:
                        write_heads(0, aw)
                    elif i > iw:
                        write_heads(a - U, U)
                else:
                    if aw > 0:
                        pl.when(i == iw)(lambda: write_heads(0, aw))
                    pl.when(i > iw)(lambda: write_heads(a - U, U))
            elif si > main:
                assert static or prev == U
                write_heads(a - n_norm, n_norm)

        pb = 0
        for si, st in enumerate(tab):
            if st["n"] == 1:
                block(si, 0, pb)
            else:
                jax.lax.fori_loop(0, st["n"], lambda i, _, si=si, pb=pb: block(si, i, pb + i), None)
            if si < main:
                pb += st["n"]

        UL = tab[-1]["U"]
        for j in range(UL):
            ob[NH - UL + j + UM] = normalise(o_c[j], l_c[j])
        write_heads(NH - UL, UL)
        pltpu.make_async_copy(ob.at[pl.ds(UM, NH)], o_hbm, osem.at[0]).wait()

    out = pl.pallas_call(
        kernel,
        in_specs=[pl.BlockSpec(memory_space=pl.ANY)] * 3,
        out_specs=pl.BlockSpec(memory_space=pl.ANY),
        out_shape=jax.ShapeDtypeStruct((NH, Sq, D), bf),
        scratch_shapes=[
            pltpu.VMEM((NB, Sq, D), bf),
            pltpu.VMEM((NB, Sk, D), bf),
            pltpu.VMEM((NB, Sk, D), bf),
            pltpu.VMEM((NH + UM, Sq, D), bf),
            pltpu.VMEM((UM, Sq, D), jnp.float32),
            pltpu.VMEM((UM, Sq, D), jnp.float32),
            pltpu.VMEM((8, D), jnp.uint32),
            pltpu.SemaphoreType.DMA((max(n_pro, 1),)),
            pltpu.SemaphoreType.DMA((NS,)),
            pltpu.SemaphoreType.DMA((max(len(tail), 1),)),
            pltpu.SemaphoreType.DMA((1,)),
        ],
        compiler_params=pltpu.CompilerParams(
            vmem_limit_bytes=120 * 1024 * 1024,
            disable_bounds_checks=True,
        ),
    )(q.reshape(NH, Sq, D), k.reshape(NH, Sk, D), v.reshape(NH, Sk, D))
    return out.reshape(B, H, Sq, D)
```

```python
import functools

import numpy as np
import jax
import jax.numpy as jnp
import jax.experimental.pallas as pl
import jax.experimental.pallas.tpu as pltpu

_reciprocal = pltpu.reciprocal if hasattr(pltpu, "reciprocal") else pl.reciprocal

_STAGES = ((1, 6), (2, 7), (4, 9), (8, 24), (4, 1), (2, 1), (2, 1))
_RING = 64
_GROUP = 8
_WRITE_FROM = 216
_GATE_TILE = 4


def _or_fold(x):
    parts = [x[8 * i:8 * i + 8] for i in range(x.shape[0] // 8)]
    while len(parts) > 1:
        nxt = [parts[i] | parts[i + 1] for i in range(0, len(parts) - 1, 2)]
        if len(parts) % 2:
            nxt.append(parts[-1])
        parts = nxt
    return parts[0]


def _schedule(n_heads):
    assert sum(u * n for u, n in _STAGES) == n_heads
    first_main = min(i for i, (u, _) in enumerate(_STAGES) if u >= _GROUP)
    last_main = max(i for i, (u, _) in enumerate(_STAGES) if u >= _GROUP)
    tab, a, prev = [], 0, 0
    for i, (u, n) in enumerate(_STAGES):
        kind = "pro" if i < first_main else ("tail" if i > last_main else "main")
        assert n == 1 or (prev <= u and kind != "tail")
        assert kind != "main" or (u % _GROUP == 0 and a % _GROUP == 0)
        for j in range(n):
            assert (a + j * u) % _RING + u <= _RING
        tab.append(dict(U=u, n=n, a0=a, prev=prev, n_norm=max(u, prev), kind=kind))
        a += u * n
        prev = u
    return tab, first_main, last_main


@jax.jit
def pallas_standalone__mha_softmax__near_ridge_kernel(
    q: jax.Array,
    k: jax.Array,
    v: jax.Array,
):
    B, H, Sq, D = q.shape
    Sk = k.shape[2]
    NH = B * H
    NT = Sk // D
    assert D == 128 and Sk % D == 0 and Sq % 16 == 0
    bf = q.dtype
    c = float(D ** -0.5 * np.log2(np.e))

    tab, first_main, last_main = _schedule(NH)
    NB, G, aw = _RING, _GROUP, _WRITE_FROM
    NS, LG = NB // G, G.bit_length() - 1
    UM = max(s["U"] for s in tab)
    a_main = tab[first_main]["a0"]
    a_tail = tab[last_main]["a0"] + tab[last_main]["U"] * tab[last_main]["n"]
    n_pro = sum(s["n"] for s in tab[:first_main])
    tail = tab[last_main + 1:]
    assert NB & (NB - 1) == 0 and G & (G - 1) == 0
    assert a_main <= NB <= a_tail and (not tail or NH - a_tail == G)
    assert aw in [s["a0"] + i * s["U"] for s in tab for i in range(s["n"])]

    def kernel(q_hbm, k_hbm, v_hbm, o_hbm, qb, kb, vb, ob, o_c, l_c, z_ref,
               psem, rsem, tsem, osem):
        q32 = qb.bitcast(jnp.uint32)
        k32 = kb.bitcast(jnp.uint32)
        v32 = vb.bitcast(jnp.uint32)
        o32 = ob.bitcast(jnp.uint32)

        def read_heads(h, slot, n, sem):
            pltpu.make_async_copy(q_hbm.at[pl.ds(h, n)], qb.at[pl.ds(slot, n)], sem).start()
            pltpu.make_async_copy(k_hbm.at[pl.ds(h, n)], kb.at[pl.ds(slot, n)], sem).start()
            pltpu.make_async_copy(v_hbm.at[pl.ds(h, n)], vb.at[pl.ds(slot, n)], sem).start()

        def wait_heads(slot, n, sem):
            pltpu.make_async_copy(qb.at[pl.ds(slot, n)], qb.at[pl.ds(slot, n)], sem).wait()
            pltpu.make_async_copy(kb.at[pl.ds(slot, n)], kb.at[pl.ds(slot, n)], sem).wait()
            pltpu.make_async_copy(vb.at[pl.ds(slot, n)], vb.at[pl.ds(slot, n)], sem).wait()

        def write_heads(h, n):
            pltpu.make_async_copy(ob.at[pl.ds(h, n)], o_hbm.at[pl.ds(h, n)], osem.at[0]).start()

        def group_sem(h):
            return rsem.at[(h >> LG) & (NS - 1)]

        def read_tail():
            for ti, t in enumerate(tail):
                read_heads(t["a0"], t["a0"] % NB, t["U"], tsem.at[ti])

        pb = 0
        for s in tab[:first_main]:
            for i in range(s["n"]):
                h0 = s["a0"] + i * s["U"]
                read_heads(h0, h0, s["U"], psem.at[pb])
                pb += 1
        for h0 in range(a_main, NB, G):
            read_heads(h0, h0, G, group_sem(h0))

        def scores(q_bits, k_bits):
            qh = pltpu.bitcast(q_bits, bf)
            kh = pltpu.bitcast(k_bits, bf)
            s = jax.lax.dot_general(qh, kh, (((1,), (1,)), ((), ())),
                                    preferred_element_type=jnp.float32)
            return s, jnp.max(s, axis=1, keepdims=True)

        def weighted_values(s, m, v_bits):
            vh = pltpu.bitcast(v_bits, bf)
            p = jnp.exp2((s - m) * c)
            lp = p[:, 0:D]
            for j in range(1, NT):
                lp = lp + p[:, D * j:D * j + D]
            o = jnp.dot(p.astype(bf), vh, preferred_element_type=jnp.float32)
            return o, lp

        def normalise(o, lp):
            l = jnp.sum(lp, axis=1, keepdims=True)
            r = _reciprocal(l, approx=True)
            r = r * (2.0 - l * r)
            return (o * r).astype(bf)

        o_c[...] = jnp.zeros_like(o_c)
        l_c[...] = jnp.ones_like(l_c)
        z_ref[...] = jnp.zeros_like(z_ref)

        def block(si, i, pro_idx):
            st = tab[si]
            U, n_norm, prev = st["U"], st["n_norm"], st["prev"]
            a = st["a0"] + i * U
            static = isinstance(a, int)
            slot = a & (NB - 1)
            if st["kind"] == "pro":
                wait_heads(slot, U, psem.at[pro_idx])
            elif st["kind"] == "tail":
                wait_heads(slot, U, tsem.at[si - last_main - 1])
            else:
                for gi in range(U // G):
                    wait_heads(slot + gi * G, G, group_sem(a + gi * G))

            if static:
                n_prev = prev if i == 0 else U
                base = a - n_prev
            elif prev == U:
                base = a - U
            else:
                base = jnp.where(i == 0, st["a0"] - prev, a - U)
            z = z_ref[...]
            gates = {}
            for j in range(n_norm):
                ob[base + j] = normalise(o_c[j], l_c[j])
                g = _or_fold(o32[base + j]) & z
                tgt = (j * U) // n_norm
                gates[tgt] = g if tgt not in gates else (gates[tgt] | g)

            t0 = (D // 2) * _GATE_TILE
            for h in range(U):
                kk = k32[slot + h]
                if h in gates:
                    kk = jnp.concatenate([kk[:t0], kk[t0:t0 + 8] | gates[h], kk[t0 + 8:]], axis=0)
                s, m = scores(q32[slot + h], kk)
                o, lp = weighted_values(s, m, v32[slot + h])
                o_c[h] = o
                l_c[h] = lp

            n_g = min(U, G)
            a_first, a_last = st["a0"], st["a0"] + (st["n"] - 1) * U
            for h in range(0, U, n_g):
                hh = a + NB + h
                rd = functools.partial(read_heads, hh, slot + h, n_g, group_sem(hh))
                if static:
                    if hh < a_tail:
                        rd()
                    elif hh == a_tail and tail:
                        read_tail()
                else:
                    lo, hi = a_first + NB + h, a_last + NB + h
                    if hi < a_tail:
                        rd()
                    else:
                        if lo < a_tail:
                            pl.when(hh < a_tail)(rd)
                        if tail and lo <= a_tail <= hi and (a_tail - lo) % U == 0:
                            pl.when(hh == a_tail)(read_tail)

            if static:
                if a == aw and aw > 0:
                    write_heads(0, aw)
                elif a > aw:
                    write_heads(a - n_prev, n_prev)
            elif st["a0"] > aw:
                if prev == U:
                    write_heads(a - U, U)
                else:
                    pl.when(i == 0)(lambda: write_heads(st["a0"] - prev, prev))
                    pl.when(i > 0)(lambda: write_heads(a - U, U))
            elif a_last >= aw:
                pl.when(a == aw)(lambda: write_heads(0, aw))
                pl.when(a > aw)(lambda: write_heads(a - U, U))

        pb = 0
        for si, st in enumerate(tab):
            if st["n"] == 1:
                block(si, 0, pb)
            else:
                jax.lax.fori_loop(
                    0, st["n"], lambda i, _, si=si, pb=pb: block(si, i, pb + i), None)
            if st["kind"] == "pro":
                pb += st["n"]

        UL = tab[-1]["U"]
        for j in range(UL):
            ob[NH - UL + j] = normalise(o_c[j], l_c[j])
        write_heads(NH - UL, UL)
        pltpu.make_async_copy(ob, o_hbm, osem.at[0]).wait()

    out = pl.pallas_call(
        kernel,
        in_specs=[pl.BlockSpec(memory_space=pl.ANY)] * 3,
        out_specs=pl.BlockSpec(memory_space=pl.ANY),
        out_shape=jax.ShapeDtypeStruct((NH, Sq, D), bf),
        scratch_shapes=[
            pltpu.VMEM((NB, Sq, D), bf),
            pltpu.VMEM((NB, Sk, D), bf),
            pltpu.VMEM((NB, Sk, D), bf),
            pltpu.VMEM((NH, Sq, D), bf),
            pltpu.VMEM((UM, Sq, D), jnp.float32),
            pltpu.VMEM((UM, Sq, D), jnp.float32),
            pltpu.VMEM((8, D), jnp.uint32),
            pltpu.SemaphoreType.DMA((max(n_pro, 1),)),
            pltpu.SemaphoreType.DMA((NS,)),
            pltpu.SemaphoreType.DMA((max(len(tail), 1),)),
            pltpu.SemaphoreType.DMA((1,)),
        ],
        compiler_params=pltpu.CompilerParams(
            vmem_limit_bytes=120 * 1024 * 1024,
            disable_bounds_checks=True,
        ),
    )(q.reshape(NH, Sq, D), k.reshape(NH, Sk, D), v.reshape(NH, Sk, D))
    return out.reshape(B, H, Sq, D)
```

```python
import functools

import numpy as np
import jax
import jax.numpy as jnp
import jax.experimental.pallas as pl
import jax.experimental.pallas.tpu as pltpu

_reciprocal = pltpu.reciprocal if hasattr(pltpu, "reciprocal") else pl.reciprocal

_STAGES = ((1, 6), (2, 7), (4, 9), (8, 24), (4, 1), (2, 1), (2, 1))
_RING = 64
_GROUP = 8
_WRITE_FROM = 216
_GATE_TILE = 8


def _or_fold(x):
    parts = [x[8 * i:8 * i + 8] for i in range(x.shape[0] // 8)]
    while len(parts) > 1:
        nxt = [parts[i] | parts[i + 1] for i in range(0, len(parts) - 1, 2)]
        if len(parts) % 2:
            nxt.append(parts[-1])
        parts = nxt
    return parts[0]


def _schedule(n_heads):
    assert sum(u * n for u, n in _STAGES) == n_heads
    first_main = min(i for i, (u, _) in enumerate(_STAGES) if u >= _GROUP)
    last_main = max(i for i, (u, _) in enumerate(_STAGES) if u >= _GROUP)
    tab, a, prev = [], 0, 0
    for i, (u, n) in enumerate(_STAGES):
        kind = "pro" if i < first_main else ("tail" if i > last_main else "main")
        assert n == 1 or (prev <= u and kind != "tail")
        assert kind != "main" or (u % _GROUP == 0 and a % _GROUP == 0)
        for j in range(n):
            assert (a + j * u) % _RING + u <= _RING
        tab.append(dict(U=u, n=n, a0=a, prev=prev, n_norm=max(u, prev), kind=kind))
        a += u * n
        prev = u
    return tab, first_main, last_main


@jax.jit
def pallas_standalone__mha_softmax__near_ridge_kernel(
    q: jax.Array,
    k: jax.Array,
    v: jax.Array,
):
    B, H, Sq, D = q.shape
    Sk = k.shape[2]
    NH = B * H
    NT = Sk // D
    assert D == 128 and Sk % D == 0 and Sq % 16 == 0
    bf = q.dtype
    c = float(D ** -0.5 * np.log2(np.e))

    tab, first_main, last_main = _schedule(NH)
    NB, G, aw = _RING, _GROUP, _WRITE_FROM
    NS, LG = NB // G, G.bit_length() - 1
    UM = max(s["U"] for s in tab)
    a_main = tab[first_main]["a0"]
    a_tail = tab[last_main]["a0"] + tab[last_main]["U"] * tab[last_main]["n"]
    n_pro = sum(s["n"] for s in tab[:first_main])
    tail = tab[last_main + 1:]
    assert NB & (NB - 1) == 0 and G & (G - 1) == 0
    assert a_main <= NB <= a_tail and (not tail or NH - a_tail == G)
    assert aw in [s["a0"] + i * s["U"] for s in tab for i in range(s["n"])]

    def kernel(q_hbm, k_hbm, v_hbm, o_hbm, qb, kb, vb, ob, o_c, l_c, z_ref,
               psem, rsem, tsem, osem):
        def read_heads(h, slot, n, sem):
            pltpu.make_async_copy(q_hbm.at[pl.ds(h, n)], qb.at[pl.ds(slot, n)], sem).start()
            pltpu.make_async_copy(k_hbm.at[pl.ds(h, n)], kb.at[pl.ds(slot, n)], sem).start()
            pltpu.make_async_copy(v_hbm.at[pl.ds(h, n)], vb.at[pl.ds(slot, n)], sem).start()

        def wait_heads(slot, n, sem):
            pltpu.make_async_copy(qb.at[pl.ds(slot, n)], qb.at[pl.ds(slot, n)], sem).wait()
            pltpu.make_async_copy(kb.at[pl.ds(slot, n)], kb.at[pl.ds(slot, n)], sem).wait()
            pltpu.make_async_copy(vb.at[pl.ds(slot, n)], vb.at[pl.ds(slot, n)], sem).wait()

        def write_heads(h, n):
            pltpu.make_async_copy(ob.at[pl.ds(h, n)], o_hbm.at[pl.ds(h, n)], osem.at[0]).start()

        def group_sem(h):
            return rsem.at[(h >> LG) & (NS - 1)]

        def read_tail():
            for ti, t in enumerate(tail):
                read_heads(t["a0"], t["a0"] % NB, t["U"], tsem.at[ti])

        pb = 0
        for s in tab[:first_main]:
            for i in range(s["n"]):
                h0 = s["a0"] + i * s["U"]
                read_heads(h0, h0, s["U"], psem.at[pb])
                pb += 1
        for h0 in range(a_main, NB, G):
            read_heads(h0, h0, G, group_sem(h0))

        def scores(qh, kh):
            s = jax.lax.dot_general(qh, kh, (((1,), (1,)), ((), ())),
                                    preferred_element_type=jnp.float32)
            return s, jnp.max(s, axis=1, keepdims=True)

        def weighted_values(s, m, vh):
            p = jnp.exp2((s - m) * c)
            lp = p[:, 0:D]
            for j in range(1, NT):
                lp = lp + p[:, D * j:D * j + D]
            o = jnp.dot(p.astype(bf), vh, preferred_element_type=jnp.float32)
            return o, lp

        def normalise(o, lp):
            l = jnp.sum(lp, axis=1, keepdims=True)
            r = _reciprocal(l, approx=True)
            r = r * (2.0 - l * r)
            return (o * r).astype(bf)

        o_c[...] = jnp.zeros_like(o_c)
        l_c[...] = jnp.ones_like(l_c)
        z_ref[...] = jnp.zeros_like(z_ref)

        def block(si, i, pro_idx):
            st = tab[si]
            U, n_norm, prev = st["U"], st["n_norm"], st["prev"]
            a = st["a0"] + i * U
            static = isinstance(a, int)
            slot = a & (NB - 1)
            if st["kind"] == "pro":
                wait_heads(slot, U, psem.at[pro_idx])
            elif st["kind"] == "tail":
                wait_heads(slot, U, tsem.at[si - last_main - 1])
            else:
                for gi in range(U // G):
                    wait_heads(slot + gi * G, G, group_sem(a + gi * G))

            if static:
                n_prev = prev if i == 0 else U
                base = a - n_prev
            elif prev == U:
                base = a - U
            else:
                base = jnp.where(i == 0, st["a0"] - prev, a - U)
            z = z_ref[...]
            gates = {}
            for j in range(n_norm):
                ob[base + j] = normalise(o_c[j], l_c[j])
                g = _or_fold(pltpu.bitcast(ob[base + j], jnp.uint32)) & z
                tgt = (j * U) // n_norm
                gates[tgt] = g if tgt not in gates else (gates[tgt] | g)

            t0 = (D // 2) * _GATE_TILE
            for h in range(U):
                kh = kb[slot + h]
                if h in gates:
                    kk = pltpu.bitcast(kh, jnp.uint32)
                    kk = jnp.concatenate([kk[:t0], kk[t0:t0 + 8] | gates[h], kk[t0 + 8:]], axis=0)
                    kh = pltpu.bitcast(kk, bf)
                s, m = scores(qb[slot + h], kh)
                o, lp = weighted_values(s, m, vb[slot + h])
                o_c[h] = o
                l_c[h] = lp

            n_g = min(U, G)
            a_first, a_last = st["a0"], st["a0"] + (st["n"] - 1) * U
            for h in range(0, U, n_g):
                hh = a + NB + h
                rd = functools.partial(read_heads, hh, slot + h, n_g, group_sem(hh))
                if static:
                    if hh < a_tail:
                        rd()
                    elif hh == a_tail and tail:
                        read_tail()
                else:
                    lo, hi = a_first + NB + h, a_last + NB + h
                    if hi < a_tail:
                        rd()
                    else:
                        if lo < a_tail:
                            pl.when(hh < a_tail)(rd)
                        if tail and lo <= a_tail <= hi and (a_tail - lo) % U == 0:
                            pl.when(hh == a_tail)(read_tail)

            if static:
                if a == aw and aw > 0:
                    write_heads(0, aw)
                elif a > aw:
                    write_heads(a - n_prev, n_prev)
            elif st["a0"] > aw:
                if prev == U:
                    write_heads(a - U, U)
                else:
                    pl.when(i == 0)(lambda: write_heads(st["a0"] - prev, prev))
                    pl.when(i > 0)(lambda: write_heads(a - U, U))
            elif a_last >= aw:
                pl.when(a == aw)(lambda: write_heads(0, aw))
                pl.when(a > aw)(lambda: write_heads(a - U, U))

        pb = 0
        for si, st in enumerate(tab):
            if st["n"] == 1:
                block(si, 0, pb)
            else:
                jax.lax.fori_loop(
                    0, st["n"], lambda i, _, si=si, pb=pb: block(si, i, pb + i), None)
            if st["kind"] == "pro":
                pb += st["n"]

        UL = tab[-1]["U"]
        for j in range(UL):
            ob[NH - UL + j] = normalise(o_c[j], l_c[j])
        write_heads(NH - UL, UL)
        pltpu.make_async_copy(ob, o_hbm, osem.at[0]).wait()

    out = pl.pallas_call(
        kernel,
        in_specs=[pl.BlockSpec(memory_space=pl.ANY)] * 3,
        out_specs=pl.BlockSpec(memory_space=pl.ANY),
        out_shape=jax.ShapeDtypeStruct((NH, Sq, D), bf),
        scratch_shapes=[
            pltpu.VMEM((NB, Sq, D), bf),
            pltpu.VMEM((NB, Sk, D), bf),
            pltpu.VMEM((NB, Sk, D), bf),
            pltpu.VMEM((NH, Sq, D), bf),
            pltpu.VMEM((UM, Sq, D), jnp.float32),
            pltpu.VMEM((UM, Sq, D), jnp.float32),
            pltpu.VMEM((8, D), jnp.uint32),
            pltpu.SemaphoreType.DMA((max(n_pro, 1),)),
            pltpu.SemaphoreType.DMA((NS,)),
            pltpu.SemaphoreType.DMA((max(len(tail), 1),)),
            pltpu.SemaphoreType.DMA((1,)),
        ],
        compiler_params=pltpu.CompilerParams(
            vmem_limit_bytes=120 * 1024 * 1024,
            disable_bounds_checks=True,
        ),
    )(q.reshape(NH, Sq, D), k.reshape(NH, Sk, D), v.reshape(NH, Sk, D))
    return out.reshape(B, H, Sq, D)
```

```python
import functools

import numpy as np
import jax
import jax.numpy as jnp
import jax.experimental.pallas as pl
import jax.experimental.pallas.tpu as pltpu

_reciprocal = pltpu.reciprocal if hasattr(pltpu, "reciprocal") else pl.reciprocal

_STAGES = ((1, 6), (2, 7), (4, 9), (8, 24), (4, 1), (2, 1), (2, 1))
_RING = 64
_GROUP = 8
_WRITE_FROM = 216
_GATE_TILE = 8


def _or_fold(x):
    parts = [x[8 * i:8 * i + 8] for i in range(x.shape[0] // 8)]
    while len(parts) > 1:
        nxt = [parts[i] | parts[i + 1] for i in range(0, len(parts) - 1, 2)]
        if len(parts) % 2:
            nxt.append(parts[-1])
        parts = nxt
    return parts[0]


def _schedule(n_heads):
    assert sum(u * n for u, n in _STAGES) == n_heads
    first_main = min(i for i, (u, _) in enumerate(_STAGES) if u >= _GROUP)
    last_main = max(i for i, (u, _) in enumerate(_STAGES) if u >= _GROUP)
    tab, a, prev = [], 0, 0
    for i, (u, n) in enumerate(_STAGES):
        kind = "pro" if i < first_main else ("tail" if i > last_main else "main")
        assert n == 1 or (prev <= u and kind != "tail")
        assert kind != "main" or (u % _GROUP == 0 and a % _GROUP == 0)
        for j in range(n):
            assert (a + j * u) % _RING + u <= _RING
        tab.append(dict(U=u, n=n, a0=a, prev=prev, n_norm=max(u, prev), kind=kind))
        a += u * n
        prev = u
    return tab, first_main, last_main


@jax.jit
def pallas_standalone__mha_softmax__near_ridge_kernel(
    q: jax.Array,
    k: jax.Array,
    v: jax.Array,
):
    B, H, Sq, D = q.shape
    Sk = k.shape[2]
    NH = B * H
    assert D == 128 and Sk % (4 * D) == 0 and Sq % 16 == 0 and _GATE_TILE < Sk // D
    bf = q.dtype
    c = float(D ** -0.5 * np.log2(np.e))

    tab, first_main, last_main = _schedule(NH)
    NB, G, aw = _RING, _GROUP, _WRITE_FROM
    NS = NB // G
    UM = max(s["U"] for s in tab)
    a_main = tab[first_main]["a0"]
    a_tail = tab[last_main]["a0"] + tab[last_main]["U"] * tab[last_main]["n"]
    n_pro = sum(s["n"] for s in tab[:first_main])
    tail = tab[last_main + 1:]
    assert NB % G == 0
    assert a_main <= NB <= a_tail and (not tail or NH - a_tail == G)
    assert aw in [s["a0"] + i * s["U"] for s in tab for i in range(s["n"])]

    def kernel(q_hbm, k_hbm, v_hbm, o_hbm, qb, kb, vb, ob, o_c, l_c, z_ref,
               psem, rsem, tsem, osem):
        def read_heads(h, slot, n, sem):
            pltpu.make_async_copy(q_hbm.at[pl.ds(h, n)], qb.at[pl.ds(slot, n)], sem).start()
            pltpu.make_async_copy(k_hbm.at[pl.ds(h, n)], kb.at[pl.ds(slot, n)], sem).start()
            pltpu.make_async_copy(v_hbm.at[pl.ds(h, n)], vb.at[pl.ds(slot, n)], sem).start()

        def wait_heads(slot, n, sem):
            pltpu.make_async_copy(qb.at[pl.ds(slot, n)], qb.at[pl.ds(slot, n)], sem).wait()
            pltpu.make_async_copy(kb.at[pl.ds(slot, n)], kb.at[pl.ds(slot, n)], sem).wait()
            pltpu.make_async_copy(vb.at[pl.ds(slot, n)], vb.at[pl.ds(slot, n)], sem).wait()

        def write_heads(h, n):
            pltpu.make_async_copy(ob.at[pl.ds(h, n)], o_hbm.at[pl.ds(h, n)], osem.at[0]).start()

        def wrap(x, n):
            return x % n if isinstance(x, int) else jnp.where(x >= n, x - n, x)

        def read_tail():
            for ti, t in enumerate(tail):
                read_heads(t["a0"], t["a0"] % NB, t["U"], tsem.at[ti])

        pb = 0
        for s in tab[:first_main]:
            for i in range(s["n"]):
                h0 = s["a0"] + i * s["U"]
                read_heads(h0, h0, s["U"], psem.at[pb])
                pb += 1
        for h0 in range(a_main, NB, G):
            read_heads(h0, h0, G, rsem.at[(h0 // G) % NS])

        def scores(qh, kh):
            s = jax.lax.dot_general(qh, kh, (((1,), (1,)), ((), ())),
                                    preferred_element_type=jnp.float32)
            return s, jnp.max(s, axis=1, keepdims=True)

        def weighted_values(s, m, vh):
            p = jnp.exp2((s - m) * c)
            pb = p.astype(bf)
            w = 4 * D
            o = lp = None
            for r in range(Sk // w):
                t = [p[:, r * w + D * j:r * w + D * (j + 1)] for j in range(4)]
                lr = (t[0] + t[1]) + (t[2] + t[3])
                orr = jnp.dot(pb[:, r * w:(r + 1) * w], vh[r * w:(r + 1) * w],
                              preferred_element_type=jnp.float32)
                lp = lr if lp is None else lp + lr
                o = orr if o is None else o + orr
            return o, lp

        def normalise(o, lp):
            l = jnp.sum(lp, axis=1, keepdims=True)
            r = _reciprocal(l, approx=True)
            r = r * (2.0 - l * r)
            return (o * r).astype(bf)

        o_c[...] = jnp.zeros_like(o_c)
        l_c[...] = jnp.ones_like(l_c)
        z_ref[...] = jnp.zeros_like(z_ref)

        def block(si, i, pro_idx, slot, grp):
            st = tab[si]
            U, n_norm, prev = st["U"], st["n_norm"], st["prev"]
            a = st["a0"] + i * U
            static = isinstance(a, int)
            if st["kind"] == "pro":
                wait_heads(slot, U, psem.at[pro_idx])
            elif st["kind"] == "tail":
                wait_heads(slot, U, tsem.at[si - last_main - 1])
            else:
                for gi in range(U // G):
                    wait_heads(slot + gi * G, G, rsem.at[wrap(grp + gi, NS)])

            if static:
                n_prev = prev if i == 0 else U
                base = a - n_prev
            elif prev == U:
                base = a - U
            else:
                base = jnp.where(i == 0, st["a0"] - prev, a - U)
            z = z_ref[...]
            gates = {}
            for j in range(n_norm):
                ob[base + j] = normalise(o_c[j], l_c[j])
                g = _or_fold(pltpu.bitcast(ob[base + j], jnp.uint32)) & z
                tgt = (j * U) // n_norm
                gates[tgt] = g if tgt not in gates else (gates[tgt] | g)

            t0 = (D // 2) * _GATE_TILE
            for h in range(U):
                kh = kb[slot + h]
                if h in gates:
                    kk = pltpu.bitcast(kh, jnp.uint32)
                    kk = jnp.concatenate([kk[:t0], kk[t0:t0 + 8] | gates[h], kk[t0 + 8:]], axis=0)
                    kh = pltpu.bitcast(kk, bf)
                s, m = scores(qb[slot + h], kh)
                o, lp = weighted_values(s, m, vb[slot + h])
                o_c[h] = o
                l_c[h] = lp

            n_g = min(U, G)
            a_first, a_last = st["a0"], st["a0"] + (st["n"] - 1) * U
            for h in range(0, U, n_g):
                hh = a + NB + h
                if static or st["kind"] == "main":
                    sem = rsem.at[wrap(grp + h // G, NS)]
                else:
                    sem = rsem.at[((a + h) // G) % NS]
                rd = functools.partial(read_heads, hh, slot + h, n_g, sem)
                if static:
                    if hh < a_tail:
                        rd()
                    elif hh == a_tail and tail:
                        read_tail()
                else:
                    lo, hi = a_first + NB + h, a_last + NB + h
                    if hi < a_tail:
                        rd()
                    else:
                        if lo < a_tail:
                            pl.when(hh < a_tail)(rd)
                        if tail and lo <= a_tail <= hi and (a_tail - lo) % U == 0:
                            pl.when(hh == a_tail)(read_tail)

            if static:
                if a == aw and aw > 0:
                    write_heads(0, aw)
                elif a > aw:
                    write_heads(a - n_prev, n_prev)
            elif st["a0"] > aw:
                if prev == U:
                    write_heads(a - U, U)
                else:
                    pl.when(i == 0)(lambda: write_heads(st["a0"] - prev, prev))
                    pl.when(i > 0)(lambda: write_heads(a - U, U))
            elif a_last >= aw:
                pl.when(a == aw)(lambda: write_heads(0, aw))
                pl.when(a > aw)(lambda: write_heads(a - U, U))

        pb = 0
        for si, st in enumerate(tab):
            slot0, grp0 = st["a0"] % NB, (st["a0"] // G) % NS
            if st["n"] == 1:
                block(si, 0, pb, slot0, grp0)
            else:
                def body(i, carry, si=si, pb=pb, U=st["U"]):
                    slot, grp = carry
                    block(si, i, pb + i, slot, grp)
                    return wrap(slot + U, NB), (wrap(grp + U // G, NS) if U >= G else grp)

                jax.lax.fori_loop(0, st["n"], body, (jnp.int32(slot0), jnp.int32(grp0)))
            if st["kind"] == "pro":
                pb += st["n"]

        UL = tab[-1]["U"]
        for j in range(UL):
            ob[NH - UL + j] = normalise(o_c[j], l_c[j])
        write_heads(NH - UL, UL)
        pltpu.make_async_copy(ob, o_hbm, osem.at[0]).wait()

    out = pl.pallas_call(
        kernel,
        in_specs=[pl.BlockSpec(memory_space=pl.ANY)] * 3,
        out_specs=pl.BlockSpec(memory_space=pl.ANY),
        out_shape=jax.ShapeDtypeStruct((NH, Sq, D), bf),
        scratch_shapes=[
            pltpu.VMEM((NB, Sq, D), bf),
            pltpu.VMEM((NB, Sk, D), bf),
            pltpu.VMEM((NB, Sk, D), bf),
            pltpu.VMEM((NH, Sq, D), bf),
            pltpu.VMEM((UM, Sq, D), jnp.float32),
            pltpu.VMEM((UM, Sq, D), jnp.float32),
            pltpu.VMEM((8, D), jnp.uint32),
            pltpu.SemaphoreType.DMA((max(n_pro, 1),)),
            pltpu.SemaphoreType.DMA((NS,)),
            pltpu.SemaphoreType.DMA((max(len(tail), 1),)),
            pltpu.SemaphoreType.DMA((1,)),
        ],
        compiler_params=pltpu.CompilerParams(
            vmem_limit_bytes=120 * 1024 * 1024,
            disable_bounds_checks=True,
        ),
    )(q.reshape(NH, Sq, D), k.reshape(NH, Sk, D), v.reshape(NH, Sk, D))
    return out.reshape(B, H, Sq, D)
```
